```python
import jax
import jax.numpy as jnp

def _softmax(x, axis=-1):
    return jax.nn.softmax(x, axis=axis)

def _gelu(x):
    return jax.nn.gelu(x, approximate=True)

def _silu(x):
    return jax.nn.silu(x)

def _sigmoid(x):
    return jax.nn.sigmoid(x)

def _layernorm(x, axis=-1, eps=1e-05):
    m = jnp.mean(x, axis=axis, keepdims=True)
    v = jnp.var(x, axis=axis, keepdims=True)
    return (x - m) / jnp.sqrt(v + eps)

def _scatter_add(tgt, idx, src, axis=0):
    return tgt.at[idx].add(src)

def _segment_sum(src, seg, n):
    return jax.ops.segment_sum(src, seg, n)

class _Rng:

    def __init__(self, key):
        self._k = key

    def _next(self):
        self._k, sub = jax.random.split(self._k)
        return sub

    def normal(self, shape):
        return jax.random.normal(self._next(), shape, dtype=jnp.bfloat16)

    def randint(self, lo, hi, shape):
        return jax.random.randint(self._next(), shape, lo, hi, dtype=jnp.int32)

    def uniform(self, shape, lo=0.0, hi=1.0):
        return jax.random.uniform(self._next(), shape, jnp.bfloat16, lo, hi)

    def permutation(self, n):
        return jax.random.permutation(self._next(), n)
kernel_name = 'adaLN_cond__ssm_conv_h3__glu_gated_bilinear__prompt'

def setup_inputs():
    _rng = _Rng(jax.random.key(int.from_bytes(__import__("os").urandom(4), "little")))
    _w = lambda a: (lambda t: t.astype(jnp.bfloat16) if jnp.issubdtype(t.dtype, jnp.floating) else t)(jnp.asarray(a))

    def _A_setup():
        B, S, D = (1, 2048, 640)
        ks = 4
        return {'q': _w((lambda *s: _rng.normal(s) * 0.05)(B, S, D)), 'k': _w((lambda *s: _rng.normal(s) * 0.05)(B, S, D)), 'v': _w((lambda *s: _rng.normal(s) * 0.05)(B, S, D)), 'shift_k': _w((lambda *s: _rng.normal(s) * 0.05)(D, ks) * 0.5), 'ssm_k': _w((lambda *s: _rng.normal(s) * 0.05)(D, S) * (1.0 / S ** 0.5)), 'ssm_D': _w((lambda *s: _rng.normal(s) * 0.05)(D))}
    _A_in = _A_setup()

    def _B_setup():
        B, S, D, F = (1, 2048, 640, 1536)
        return {'x': _w((lambda *s: _rng.normal(s) * 0.05)(B, S, D)), 'w_gate': _w((lambda *s: _rng.normal(s) * 0.05)(D, F) * D ** (-0.5)), 'w_up': _w((lambda *s: _rng.normal(s) * 0.05)(D, F) * D ** (-0.5)), 'w_down': _w((lambda *s: _rng.normal(s) * 0.05)(F, D) * F ** (-0.5))}
    _B_in = _B_setup()
    return {'A_q': _A_in['q'], 'A_k': _A_in['k'], 'A_v': _A_in['v'], 'A_shift_k': _A_in['shift_k'], 'A_ssm_k': _A_in['ssm_k'], 'A_ssm_D': _A_in['ssm_D'], 'B_x': _B_in['x'], 'B_w_gate': _B_in['w_gate'], 'B_w_up': _B_in['w_up'], 'B_w_down': _B_in['w_down'], 'c': _w((lambda *s: _rng.normal(s) * 0.05)(1, 640)), 'w_mod': _w((lambda *s: _rng.normal(s) * 0.05)(640, 6 * 640) * 640 ** (-0.5))}

def reference(A_q, A_k, A_v, A_shift_k, A_ssm_k, A_ssm_D, B_x, B_w_gate, B_w_up, B_w_down, c, w_mod):

    def _A_ref(q, k, v, shift_k, ssm_k, ssm_D):
        B, S, D = q.shape
        ks = shift_k.shape[-1]
        k_pad = jnp.pad(k, ((0, 0), (ks - 1, 0), (0, 0)))
        k_shift = jnp.zeros_like(k)
        for t in range(ks):
            k_shift = k_shift + k_pad[:, t:t + S, :] * shift_k[:, ks - 1 - t][None, None, :]
        kv = k_shift * v
        L = 2 * S
        kv_pad = jnp.pad(kv, ((0, 0), (0, S), (0, 0)))
        kf_pad = jnp.pad(ssm_k, ((0, 0), (0, S)))
        kv_f = (lambda x, axes=(-2, -1): jnp.fft.rfft2(x.astype(jnp.float32), axes=axes))(kv_pad[:, None, :, :], axes=(1, 2))
        kf_f = (lambda x, axes=(-2, -1): jnp.fft.rfft2(x.astype(jnp.float32), axes=axes))(kf_pad[:, None, :], axes=(1, 2))
        kf_f = (lambda x, *d: x.transpose(*d))(kf_f, 1, 2, 0)
        y_f = kv_f * kf_f[None, :, :, :]
        y = (lambda x, s, axes=(-2, -1): jnp.fft.irfft2(x, s=s, axes=axes).astype(jnp.bfloat16))(y_f, (1, L), axes=(1, 2))[:, 0, :S, :]
        y = y + kv * ssm_D[None, None, :]
        return q * y

    def _B_ref(x, w_gate, w_up, w_down):
        g = jnp.einsum('bsd,df->bsf', x, w_gate)
        u = jnp.einsum('bsd,df->bsf', x, w_up)
        h = g * u
        return jnp.einsum('bsf,fd->bsd', h, w_down)
    x = A_q
    mod = (_silu(c) @ w_mod).reshape(c.shape[0], 6, 1, -1)
    sa, ca, ga, sb, cb, gb = (mod[:, 0].copy(), mod[:, 1].copy(), mod[:, 2].copy(), mod[:, 3].copy(), mod[:, 4].copy(), mod[:, 5].copy())
    h = _layernorm(x, axis=-1) * (1 + ca) + sa
    x = x + ga * _A_ref(h, A_k, A_v, A_shift_k, A_ssm_k, A_ssm_D)
    h = _layernorm(x, axis=-1) * (1 + cb) + sb
    x = x + gb * _B_ref(h, B_w_gate, B_w_up, B_w_down)
    return x
```

```python
import functools
import numpy as np
import jax
import jax.numpy as jnp
from jax import lax
import jax.experimental.pallas as pl
import jax.experimental.pallas.tpu as pltpu

S, D, FD = 2048, 640, 1536
P = 128
NB = S // P
BM = 256
BPS = BM // P
NS = S // BM
NL = D // 128
HALO = 16
EPS = 1e-5
F32, BF16 = jnp.float32, jnp.bfloat16
FC = 512
NFC = FD // FC
MAC_SEG = 8


def _dft_consts():
    f = np.concatenate([np.arange(0, P, 2), np.arange(1, P, 2)]).astype(np.float64)
    n = np.arange(P, dtype=np.float64)
    ang = np.pi * (2 * f[:, None] + 1) * n[None, :] / (2 * P)
    fwd = np.concatenate([np.cos(ang), -np.sin(ang)], axis=0)
    inv = fwd.T / P
    return fwd.astype(np.float32), inv.astype(np.float32)


def _ln(x):
    m = jnp.mean(x, axis=-1, keepdims=True)
    xc = x - m
    v = jnp.mean(xc * xc, axis=-1, keepdims=True)
    return xc * lax.rsqrt(v + EPS)


class _Sched:
    def __init__(self, mask):
        self.mask = mask
        self.q = {}
        self.t = 0

    def add(self, segs, t0, t1):
        n = len(segs)
        for s, fn in enumerate(segs):
            self.q.setdefault(t0 + (s * (t1 - t0)) // n, []).append(fn)

    def fire(self, p):
        segs = self.q.pop(self.t, [])
        self.t += 1
        nrg, nlt = p.shape[0] // 8, p.shape[1] // 128
        for j, fn in enumerate(segs):
            rg = (j * nrg) // len(segs)
            lt = j % min(nlt, 4)
            fn(jnp.where(self.mask, p[rg * 8:rg * 8 + 8, lt * 128:(lt + 1) * 128], 0.0))

    def flush(self):
        for t in sorted(self.q):
            for fn in self.q[t]:
                fn(None)
        self.q = {}


def _kernel(q_h, k_h, v_h, shk_h, s_h, dv_h, wg_h, wu_h, wd_h, c_h, wm_h, ff_h, fi_h, o_h,
            q_v, k_v, v_v, s_v, wg_v, wu_v, wd_v, wm_v, shk_v, dv_v, c_v, ff_v, fi_v,
            K_s, W_s, U_s, Z_s, kv_s, y_s, hb_v, x1_v, o_v, sems):
    nsem = [0]

    def mk(src, dst):
        c = pltpu.make_async_copy(src, dst, sems.at[nsem[0]])
        nsem[0] += 1
        return c

    def blk(i):
        r = pl.ds(i * BM, BM)
        return dict(
            s=mk(s_h.at[:, r], s_v.at[:, r]),
            k=mk(k_h.at[r], k_v.at[pl.ds(HALO + i * BM, BM)]),
            v=mk(v_h.at[r], v_v.at[r]),
            q=mk(q_h.at[r], q_v.at[r]),
        )

    small = [mk(shk_h, shk_v), mk(dv_h, dv_v), mk(c_h, c_v), mk(ff_h, ff_v), mk(fi_h, fi_v)]
    blks = [blk(i) for i in range(NS)]
    wm = [mk(wm_h.at[:, pl.ds(j * D, D)], wm_v.at[:, pl.ds(j * D, D)]) for j in range(6)]
    wch = []
    for j in range(NFC):
        cs = pl.ds(j * FC, FC)
        wch.append([mk(wg_h.at[:, cs], wg_v.at[:, cs]), mk(wu_h.at[:, cs], wu_v.at[:, cs]), mk(wd_h.at[cs], wd_v.at[cs])])
    outs = [mk(o_v.at[pl.ds(i * BM, BM)], o_h.at[pl.ds(i * BM, BM)]) for i in range(NS)]

    for c in small: c.start()
    for n in "skv": blks[0][n].start()
    for n in "skv": blks[1][n].start()
    for j in range(5): wm[j].start()
    blks[0]["q"].start()
    for c in wch[0]: c.start()
    blks[1]["q"].start()
    for n in "skv": blks[2][n].start()
    for j in range(1, NFC):
        for c in wch[j]: c.start()
    wm[5].start()
    for i in range(2, NS):
        blks[i]["q"].start()
        if i + 1 < NS:
            for n in "skv": blks[i + 1][n].start()

    k_v[0:HALO, :] = jnp.zeros((HALO, D), BF16)

    for c in small: c.wait()
    ff = ff_v[...]
    fi = fi_v[...]
    never = ff_v[0:8, :].astype(F32) > 2.0
    eye = (lax.broadcasted_iota(jnp.int32, (8, 4), 0) == lax.broadcasted_iota(jnp.int32, (8, 4), 1)).astype(BF16)
    taps = lax.dot_general(eye, shk_v[...], (((1,), (1,)), ((), ())), preferred_element_type=F32)
    dvec = dv_v[...].astype(F32)

    def kv_segs(i):
        segs = []
        R = 64
        for l in range(NL):
            ls = slice(l * 128, (l + 1) * 128)
            for r in range(0, BM, R):
                def seg(trig, ls=ls, r=r):
                    r0 = i * BM + r
                    kk = k_v[r0 + HALO - 8:r0 + HALO + R, ls].astype(F32)
                    acc = kk[8:, :] * taps[0:1, ls]
                    if trig is not None:
                        acc = acc + jnp.concatenate([trig] * (R // 8), axis=0)
                    for j in range(1, 4):
                        acc = acc + pltpu.roll(kk, j, axis=0)[8:, :] * taps[j:j + 1, ls]
                    kv_s[r:r + R, ls] = (acc * v_v[r0:r0 + R, ls].astype(F32)).astype(BF16)
                segs.append(seg)
        return segs

    def mac_segs(i):
        segs = []
        cs = [i * BPS + b for b in range(BPS)]
        nm = max(cs) + 1
        nseg = -(-nm // MAC_SEG)
        for l in range(NL):
            ls = slice(l * 128, (l + 1) * 128)
            for r2 in range(P // 16):
                res = {c: [[], []] for c in cs}
                for r in (2 * r2, 2 * r2 + 1):
                    st = dict(acc={}, ld={})
                    for sg in range(nseg):
                        def seg(trig, ls=ls, r=r, r2=r2, sg=sg, st=st, res=res):
                            acc, ld = st["acc"], st["ld"]

                            def get(ref, name, idx, im):
                                key = (name, idx, im)
                                if key not in ld:
                                    ld[key] = ref[idx, im * P + r * 8: im * P + r * 8 + 8, ls]
                                return ld[key]
                            for m in range(sg * MAC_SEG, min(nm, (sg + 1) * MAC_SEG)):
                                kr, ki = get(K_s, "k", m, 0), get(K_s, "k", m, 1)
                                if trig is not None and m == sg * MAC_SEG:
                                    kr = kr + trig
                                    ki = ki + trig
                                for c in cs:
                                    a = c - m
                                    if a < 0:
                                        continue
                                    wr, wi = get(W_s, "w", a, 0), get(W_s, "w", a, 1)
                                    tr = kr * wr - ki * wi
                                    ti = kr * wi + ki * wr
                                    acc[c] = (tr, ti) if c not in acc else (acc[c][0] + tr, acc[c][1] + ti)
                            if sg == nseg - 1:
                                for c in cs:
                                    res[c][0].append(acc[c][0]); res[c][1].append(acc[c][1])
                                if r == 2 * r2 + 1:
                                    for c in cs:
                                        for im in range(2):
                                            Z_s[c, im * P + r2 * 16: im * P + r2 * 16 + 16, ls] = (
                                                jnp.concatenate(res[c][im], axis=0).astype(BF16))
                        segs.append(seg)
        return segs

    def pre_segs(i, md):
        segs = []
        R = 16
        for r in range(0, BM, R):
            def seg(trig, r=r):
                r0 = i * BM + r
                x = q_v[r0:r0 + R, :].astype(F32)
                if trig is not None:
                    x = x + jnp.concatenate([jnp.concatenate([trig] * NL, axis=1)] * (R // 8), axis=0)
                h = _ln(x) * md["ca1"] + md["sa"]
                x1 = x + md["ga"] * (h * y_s[r0:r0 + R, :])
                hb = _ln(x1) * md["cb1"] + md["sb"]
                x1_v[r0:r0 + R, :] = x1
                hb_v[r0:r0 + R, :] = hb.astype(BF16)
            segs.append(seg)
        return segs

    def dft_k(i, sch):
        for b in range(BPS):
            a = i * BPS + b
            Kf = lax.dot_general(ff, s_v[:, a * P:(a + 1) * P], (((1,), (1,)), ((), ())), preferred_element_type=F32)
            sch.fire(Kf)
            if a == 0:
                K_s[a, 0:P, :] = Kf[0:P] + dvec
                K_s[a, P:2 * P, :] = Kf[P:]
            else:
                K_s[a] = Kf

    def dft_u(i, sch):
        for b in range(BPS):
            a = i * BPS + b
            U = jnp.dot(ff, kv_s[b * P:(b + 1) * P, :], preferred_element_type=F32)
            sch.fire(U)
            if a == 0:
                W_s[a] = U
            else:
                H = P // 2
                up = U_s[...]
                W_s[a, 0 * H:1 * H, :] = U[0 * H:1 * H] - up[2 * H:3 * H]
                W_s[a, 1 * H:2 * H, :] = U[1 * H:2 * H] + up[3 * H:4 * H]
                W_s[a, 2 * H:3 * H, :] = U[2 * H:3 * H] + up[0 * H:1 * H]
                W_s[a, 3 * H:4 * H, :] = U[3 * H:4 * H] - up[1 * H:2 * H]
            U_s[...] = U

    def inv(i, sch):
        for b in range(BPS):
            c = i * BPS + b
            y = jnp.dot(fi, Z_s[c], preferred_element_type=F32)
            sch.fire(y)
            y_s[c * P:(c + 1) * P, :] = y

    def mod_row(j):
        wm[j].wait()
        r = jnp.dot(sc, wm_v[:, j * D:(j + 1) * D], preferred_element_type=F32)
        return r[0:1, :]

    NMICRO = NFC * 2 * (D // 128) * (FC // 512)

    def ffn(i, md, sch, first):
        r0 = i * BM
        hb = hb_v[r0:r0 + BM, :]
        acc = None
        for j in range(NFC):
            if first:
                wch[j][0].wait(); wch[j][1].wait()
            gu = []
            for wv in (wg_v, wu_v):
                s = None
                for k in range(D // 128):
                    p = jnp.dot(hb[:, k * 128:(k + 1) * 128], wv[k * 128:(k + 1) * 128, j * FC:(j + 1) * FC],
                                preferred_element_type=F32)
                    sch.fire(p)
                    s = p if s is None else s + p
                gu.append(s)
            hh = (gu[0] * gu[1]).astype(BF16)
            if first:
                wch[j][2].wait()
            t = jnp.dot(hh, wd_v[j * FC:(j + 1) * FC, :], preferred_element_type=F32)
            acc = t if acc is None else acc + t
        if first:
            md["gb"] = mod_row(5)
        o_v[r0:r0 + BM, :] = (x1_v[r0:r0 + BM, :] + md["gb"] * acc).astype(BF16)
        outs[i].start()

    cf = c_v[...].astype(F32)
    sc = jnp.broadcast_to((cf * jax.nn.sigmoid(cf)).astype(BF16), (16, D))
    sch = _Sched(never)
    for i in range(2):
        for n in "skv": blks[i][n].wait()
        for fn in kv_segs(i): fn(None)
        dft_k(i, sch)
        dft_u(i, sch)
        for fn in mac_segs(i): fn(None)
        if i == 0:
            inv(0, sch)
    md = {}
    md["sa"] = mod_row(0)
    md["ca1"] = 1.0 + mod_row(1)
    md["ga"] = mod_row(2)
    md["sb"] = mod_row(3)
    md["cb1"] = 1.0 + mod_row(4)
    blks[0]["q"].wait()
    for fn in pre_segs(0, md): fn(None)

    for i in range(NS):
        sch = _Sched(never)
        t = 0
        if i + 1 < NS:
            blks[i + 1]["q"].wait()
        if i + 2 < NS:
            for n in "skv": blks[i + 2][n].wait()
        has_dft, has_inv = i + 2 < NS, i + 1 < NS
        t_ffn = (BPS if has_dft else 0) + (BPS if has_inv else 0) + (BPS if has_dft else 0)
        if has_dft:
            sch.add(kv_segs(i + 2), 0, 2 * BPS)
        if has_inv:
            sch.add(pre_segs(i + 1, md), t_ffn, t_ffn + NMICRO)
        if has_dft:
            sch.add(mac_segs(i + 2), t_ffn, t_ffn + NMICRO)
        if has_dft:
            dft_k(i + 2, sch)
        if has_inv:
            inv(i + 1, sch)
        if has_dft:
            dft_u(i + 2, sch)
        ffn(i, md, sch, i == 0)
        assert not sch.q
    for o in outs:
        o.wait()


def _call(q, k, v, shk, s, dv, wg, wu, wd, c, wm):
    ff, fi = _dft_consts()
    ff = jnp.asarray(ff, dtype=BF16)
    fi = jnp.asarray(fi, dtype=BF16)
    any_ = pl.BlockSpec(memory_space=pl.ANY)
    vm = pltpu.VMEM
    return pl.pallas_call(
        _kernel,
        in_specs=[any_] * 13,
        out_specs=any_,
        out_shape=jax.ShapeDtypeStruct((S, D), BF16),
        scratch_shapes=[
            vm((S, D), BF16), vm((HALO + S, D), BF16), vm((S, D), BF16), vm((D, S), BF16),
            vm((D, FD), BF16), vm((D, FD), BF16), vm((FD, D), BF16), vm((D, 6 * D), BF16),
            vm((D, 4), BF16), vm((1, D), BF16), vm((1, D), BF16), vm((2 * P, P), BF16), vm((P, 2 * P), BF16),
            vm((NB, 2 * P, D), F32), vm((NB, 2 * P, D), F32), vm((2 * P, D), F32), vm((NB, 2 * P, D), BF16),
            vm((BM, D), BF16), vm((S, D), F32),
            vm((S, D), BF16), vm((S, D), F32), vm((S, D), BF16),
            pltpu.SemaphoreType.DMA((80,)),
        ],
        compiler_params=pltpu.CompilerParams(vmem_limit_bytes=100 * 1024 * 1024),
    )(q, k, v, shk, s, dv, wg, wu, wd, c, wm, ff, fi)


@jax.jit
def pallas_adaLN_cond__ssm_conv_h3__glu_gated_bilinear__prompt_kernel(
        A_q, A_k, A_v, A_shift_k, A_ssm_k, A_ssm_D, B_x, B_w_gate, B_w_up, B_w_down, c, w_mod):
    out = _call(A_q.reshape(S, D), A_k.reshape(S, D), A_v.reshape(S, D), A_shift_k, A_ssm_k,
                A_ssm_D.reshape(1, D), B_w_gate, B_w_up, B_w_down, c, w_mod)
    return out.reshape(1, S, D)
```

```python
import contextlib, os
import numpy as np
import jax
import jax.numpy as jnp
from jax import lax
import jax.experimental.pallas as pl
import jax.experimental.pallas.tpu as pltpu

S, D, FD = 2048, 640, 1536
P = 128
NB = S // P
BM = 256
NS = S // BM
NL = D // 128
HALO = 16
EPS = 1e-5
F32, BF16 = jnp.float32, jnp.bfloat16
FC = 512
NFC = FD // FC
TAIL = int(os.environ.get('TAIL', 1))
PTAIL = int(os.environ.get('PTAIL', 4))
KRAW = int(os.environ.get('KRAW', 1))
NSLOT = int(os.environ.get('NSLOT', 8))
PRE_LAG = float(os.environ.get('PRE_LAG', 2))


def _dft_consts():
    f = np.concatenate([np.arange(0, P, 2), np.arange(1, P, 2)]).astype(np.float64)
    w = np.pi * (2 * f[:, None] + 1) / (2 * P)
    n = np.arange(P, dtype=np.float64)[None, :]
    mid = (P - 1) / 2
    fk = np.concatenate([np.cos(w * n), -np.sin(w * n)], axis=0)
    fu = np.concatenate([np.cos(w * (n - mid)), -np.sin(w * (n - mid))], axis=0)
    tau = n[:, P // 2:] - mid
    fi = np.concatenate([np.cos(w * tau).T, np.sin(w * tau).T], axis=0) / P
    return fk.astype(np.float32), fu.astype(np.float32), fi.astype(np.float32)


def _al(x, m):
    return x if isinstance(x, int) else pl.multiple_of(x, m)


def _rows(start, n, m=16):
    return pl.ds(_al(start, m), n)


def _min(a, b):
    return min(a, b) if isinstance(a, int) else jnp.minimum(a, b)


class _Sched:
    def __init__(self, mask, dur=()):
        self.mask = mask
        self.dur = list(dur)
        self.load = [0.0] * len(self.dur)
        self.q = {}
        self.t = 0

    def add(self, segs, t0, t1, cost):
        total = cost * len(segs)
        lo, hi = 0.0, 1e3
        for _ in range(50):
            mid = (lo + hi) / 2
            room = sum(max(0.0, mid * self.dur[t] - self.load[t]) for t in range(t0, t1))
            lo, hi = (lo, mid) if room >= total else (mid, hi)
        t, left = t0, max(0.0, hi * self.dur[t0] - self.load[t0])
        for fn in segs:
            while left < cost / 2 and t + 1 < t1:
                t += 1
                left += max(0.0, hi * self.dur[t] - self.load[t])
            self.q.setdefault(t, []).append(fn)
            self.load[t] += cost
            left -= cost

    def fire(self, p):
        segs = self.q.pop(self.t, [])
        self.t += 1
        nrg, nlt = p.shape[0] // 8, p.shape[1] // 128
        for j, fn in enumerate(segs):
            rg = (j * nrg) // len(segs)
            lt = j % min(nlt, 4)
            fn(jnp.where(self.mask, p[rg * 8:rg * 8 + 8, lt * 128:(lt + 1) * 128], 0.0))


def scope(name):
    return jax.named_scope(name) if os.environ.get("SCOPES") else contextlib.nullcontext()


def _kernel(q_h, k_h, v_h, shk_h, s_h, dv_h, wg_h, wu_h, wd_h, c_h, wm_h, ff_h, fu_h, fi_h, z_s, o_h,
            q_v, k_v, v_v, s_v, wg_v, wu_v, wd_v, wm_v, shk_v, dv_v, c_v, ff_v, fu_v, fi_v,
            K_s, W_s, Zl_s, Z_s, Zp_s, kv_s, y_s, hb_v, x1_v, o_v, sems, osem):
    nsem = [0]
    STOP = int(os.environ.get('STOP_AFTER', NS))

    def mk(src, dst):
        c = pltpu.make_async_copy(src, dst, sems.at[nsem[0]])
        nsem[0] += 1
        return c

    def qq(i):
        r = pl.ds(i * BM, BM)
        return [mk(q_h.at[r], q_v.at[r])]

    def skv(i):
        r = pl.ds(i * BM, BM)
        return ([mk(s_h.at[:, pl.ds((2 * i + b) * P, P)], s_v.at[2 * i + b]) for b in range(2)]
                + [mk(k_h.at[r], k_v.at[pl.ds(HALO + i * BM, BM)]), mk(v_h.at[r], v_v.at[r])])

    def out_copy(i):
        r = _rows(i * BM, BM)
        return pltpu.make_async_copy(o_v.at[r], o_h.at[r], osem.at[i])

    small = [mk(shk_h, shk_v), mk(dv_h, dv_v), mk(c_h, c_v), mk(ff_h, ff_v), mk(fu_h, fu_v), mk(fi_h, fi_v)]
    Q = [qq(i) for i in range(NS)]
    X = [skv(i) for i in range(NS)]
    wm = [mk(wm_h.at[:, pl.ds(j * D, D)], wm_v.at[:, pl.ds(j * D, D)]) for j in range(6)]
    gu = {}
    for j in range(NFC):
        for h in range(2 if j == 0 else 1):
            cs = pl.ds(j * FC + h * FC // 2, FC // 2 if j == 0 else FC)
            gu[j, h] = [mk(wg_h.at[:, cs], wg_v.at[:, cs]), mk(wu_h.at[:, cs], wu_v.at[:, cs])]
    dn = [mk(wd_h.at[pl.ds(j * FC, FC)], wd_v.at[pl.ds(j * FC, FC)]) for j in range(NFC)]

    order = (small + X[0] + X[1] + wm[:5] + Q[0] + Q[1] + gu[0, 0] + gu[0, 1] + [dn[0]] + X[2] + gu[1, 0] + [dn[1]]
             + X[3] + gu[2, 0] + [dn[2], wm[5]] + Q[2] + X[4] + Q[3])
    for i in range(4, NS):
        order += Q[i] + (X[i + 1] if i + 1 < NS else [])
    for c in order:
        c.start()
    rest = [c for i in range(3, NS) for c in Q[i]] + [c for i in range(5, NS) for c in X[i]]

    k_v[0:HALO, :] = jnp.zeros((HALO, D), BF16)
    z0 = z_s[0]
    K_s[NB + z0] = jnp.zeros((3, P, D), F32)
    W_s[NB + z0] = jnp.zeros((3, P, D), F32)

    for c in small: c.wait()
    ff, fu = ff_v[...], fu_v[...]
    fic, fis = fi_v[0:P // 2, :], fi_v[P // 2:, :]
    never = ff_v[0:8, :].astype(F32) > 2.0
    rev8 = 7 - lax.broadcasted_iota(jnp.int32, (8, 128), 0)
    taps = shk_v[...].astype(F32)
    dvec = dv_v[...].astype(F32).reshape(1, D)

    def kv_segs(i, slot):
        segs = []
        R = 64
        for l in range(NL):
            ls = slice(l * 128, (l + 1) * 128)
            for r in range(0, BM, R):
                def seg(trig, ls=ls, r=r):
                    kk = k_v[_rows(i * BM + r + HALO - 8, 8 + R, 8), ls].astype(F32)
                    acc = kk[8:, :] * taps[0:1, ls]
                    if trig is not None:
                        acc = acc + jnp.concatenate([trig] * (R // 8), axis=0)
                    for j in range(1, 4):
                        acc = acc + pltpu.roll(kk, j, axis=0)[8:, :] * taps[j:j + 1, ls]
                    kv_s[slot, r:r + R, ls] = (acc * v_v[_rows(i * BM + r, R), ls].astype(F32)).astype(BF16)
                segs.append(seg)
        return segs

    def mac_segs(j, ts, final, resume):
        segs = []
        static = isinstance(j, int)

        def kidx(t, e):
            return 2 * t + e if static or t <= 4 else jnp.where(t <= j, 2 * t + e, NB)

        def widx(t, d):
            a = 2 * (j - t) + d
            if static:
                return a if a >= 0 else None
            return a if (t <= 4 and d >= 0) or t < 4 else jnp.where(a >= 0, a, NB)
        kix = {(t, e): kidx(t, e) for t in ts for e in range(2)}
        wix = {(t, d): widx(t, d) for t in ts for d in (-1, 0, 1)}
        for l in range(NL):
            ls = slice(l * 128, (l + 1) * 128)
            for r2 in range(P // 16):
                sts = [dict(), dict()]
                for gi, t in enumerate(ts):
                    def seg(trig, ls=ls, r2=r2, t=t, sts=sts, last=gi == len(ts) - 1):
                        outv = [[], []]
                        for h in range(2):
                            rows = slice((2 * r2 + h) * 8, (2 * r2 + h) * 8 + 8)
                            acc = sts[h]
                            ww = {d: [W_s[wix[t, d], x, rows, ls] for x in range(3)]
                                  for d in (-1, 0, 1) if wix[t, d] is not None}
                            for e in range(2):
                                if KRAW:
                                    ka, kb = [K_s[kix[t, e], x, rows, ls] for x in range(2)]
                                    if trig is not None:
                                        ka, kb = ka + trig, kb + trig
                                    kk = [ka + kb, ka, kb]
                                else:
                                    kk = [K_s[kix[t, e], x, rows, ls] for x in range(3)]
                                    if trig is not None and (e == 0 or os.environ.get('TIE6')):
                                        kk = [v + trig for v in kk]
                                for b in range(2):
                                    if b - e in ww:
                                        pr = [kk[x] * ww[b - e][x] for x in range(3)]
                                        acc[b] = pr if b not in acc else [acc[b][x] + pr[x] for x in range(3)]
                            if not last:
                                continue
                            z = []
                            for b in range(2):
                                re, im = acc[b][0] - acc[b][2], acc[b][0] + acc[b][1]
                                if resume:
                                    re = re + Zp_s[2 * b + z0, rows, ls]
                                    im = im + Zp_s[2 * b + 1 + z0, rows, ls]
                                z.append((re, im))
                            if final:
                                def shifted(cur, prev):
                                    if (2 * r2 + h) * 8 < P // 2:
                                        return cur[0] - prev[1], cur[1] + prev[0]
                                    return cur[0] + prev[1], cur[1] - prev[0]
                                z1 = shifted(z[1], z[0])
                                if static and j == 0:
                                    z0v = z[0]
                                else:
                                    z0v = shifted(z[0], (Zl_s[z0, rows, ls], Zl_s[1 + z0, rows, ls]))
                                Zl_s[z0, rows, ls] = z[1][0]
                                Zl_s[1 + z0, rows, ls] = z[1][1]
                                z = [z0v, z1]
                            for b in range(2):
                                outv[b].append(z[b])
                        if last:
                            rows = slice(r2 * 16, r2 * 16 + 16)
                            for b in range(2):
                                for x in range(2):
                                    val = jnp.concatenate([outv[b][0][x], outv[b][1][x]], axis=0)
                                    if final:
                                        Z_s[b + z0, x * P + r2 * 16:x * P + r2 * 16 + 16, ls] = val.astype(BF16)
                                    else:
                                        Zp_s[2 * b + x + z0, rows, ls] = val
                    segs.append(seg)
        return segs

    def tie(x, trig):
        if trig is None:
            return x
        t = jnp.concatenate([trig] * (x.shape[0] // 8), axis=0)
        return jnp.concatenate([x[:, :128] + t, x[:, 128:]], axis=1)

    def pre_segs(i, dst):
        R = 16
        chains = []
        for r in range(0, BM, R):
            st = {}

            def a(trig, r=r, st=st):
                st["x"] = tie(q_v[_rows(i * BM + r, R), :].astype(F32), trig)
                st["m"] = jnp.mean(st["x"], axis=-1, keepdims=True)

            def b(trig, st=st):
                st["xc"] = tie(st["x"], trig) - st["m"]
                st["v"] = jnp.mean(st["xc"] * st["xc"], axis=-1, keepdims=True)

            def c(trig, r=r, st=st):
                h = tie(st["xc"], trig) * lax.rsqrt(st["v"] + EPS) * md["ca1"] + md["sa"]
                st["x1"] = st["x"] + md["ga"] * (h * y_s[z0, r:r + R, :])
                x1_v[_rows(dst * BM + r, R), :] = st["x1"]
                st["m1"] = jnp.mean(st["x1"], axis=-1, keepdims=True)

            def d(trig, st=st):
                st["xc1"] = tie(st["x1"], trig) - st["m1"]
                st["v1"] = jnp.mean(st["xc1"] * st["xc1"], axis=-1, keepdims=True)

            def e(trig, r=r, st=st):
                hb = tie(st["xc1"], trig) * lax.rsqrt(st["v1"] + EPS) * md["cb1"] + md["sb"]
                hb_v[_rows(dst * BM + r, R), :] = hb.astype(BF16)
            chains.append([a, b, c, d, e])
        order = sorted((g + PRE_LAG * s, -s, g) for g in range(len(chains)) for s in range(5))
        return [chains[g][-ns] for _, ns, g in order]

    def dft_jobs(i, slot):
        def kjob(sch, b):
            a = 2 * i + b
            Kf = lax.dot_general(ff, s_v[a], (((1,), (1,)), ((), ())), preferred_element_type=F32)
            kr, ki = Kf[0:P], Kf[P:]
            if isinstance(a, int) and a == 0:
                kr = kr + dvec
            if KRAW:
                K_s[a + z0, 0] = kr
                K_s[a + z0, 1] = ki
            else:
                K_s[a + z0, 0] = kr + ki
                K_s[a + z0, 1] = kr
                K_s[a + z0, 2] = ki

        def ujob(sch, b):
            a = 2 * i + b
            U = jnp.dot(fu, kv_s[slot, b * P:(b + 1) * P, :], preferred_element_type=F32)
            wr, wi = U[0:P], U[P:]
            W_s[a + z0, 0] = wr
            W_s[a + z0, 1] = wi - wr
            W_s[a + z0, 2] = wr + wi
        return [lambda sch, b=b, f=f: f(sch, b) for f in (kjob, ujob) for b in range(2)]

    def inv_jobs():
        def job(sch, b):
            ye = jnp.dot(fic, Z_s[b + z0, 0:P, :], preferred_element_type=F32)
            yo = jnp.dot(fis, Z_s[b + z0, P:2 * P, :], preferred_element_type=F32)
            y_s[z0, b * P + P // 2:(b + 1) * P, :] = ye - yo
            lo = ye + yo
            for g in range(P // 16):
                src = slice((P // 16 - 1 - g) * 8, (P // 16 - g) * 8)
                y_s[z0, b * P + g * 8:b * P + g * 8 + 8, :] = jnp.concatenate(
                    [jnp.take_along_axis(lo[src, l * 128:(l + 1) * 128], rev8, axis=0) for l in range(NL)], axis=1)
        return [lambda sch, b=b: job(sch, b) for b in range(2)]

    def mod_row(j):
        r = jnp.dot(sc, wm_v[:, j * D:(j + 1) * D], preferred_element_type=F32)
        return r[0:1, :]

    def ffn_jobs(i, acc):
        st = {}
        jobs = []
        for j in range(NFC):
            for n in range(FC // 128):
                cs = slice(j * FC + n * 128, j * FC + (n + 1) * 128)

                def gate(sch, j=j, n=n, cs=cs):
                    if n == 0:
                        st["hh"] = []
                        if j == 0:
                            st["hb"] = hb_v[_rows(i * BM, BM), :]
                    if os.environ.get("HB_RELOAD"):
                        st["hb"] = hb_v[_rows(i * BM, BM), :]
                    st["g"] = jnp.dot(st["hb"], wg_v[:, cs], preferred_element_type=F32)
                    sch.fire(st["g"])

                def up(sch, cs=cs):
                    if os.environ.get("HB_RELOAD") == "2":
                        st["hb"] = hb_v[_rows(i * BM, BM), :]
                    u = jnp.dot(st["hb"], wu_v[:, cs], preferred_element_type=F32)
                    sch.fire(u)
                    st["hh"].append(st["g"] * u)
                jobs += [gate, up]
            for n in range(NL):
                def down(sch, j=j, n=n):
                    if n == 0:
                        st["h"] = jnp.concatenate(st["hh"], axis=1).astype(BF16)
                    t = jnp.dot(st["h"], wd_v[j * FC:(j + 1) * FC, n * 128:(n + 1) * 128], preferred_element_type=F32)
                    sch.fire(t)
                    acc[n] = t if acc[n] is None else acc[n] + t
                jobs.append(down)
        return jobs

    def ffn_out(i, acc):
        r = _rows(i * BM, BM)
        o_v[r, :] = (x1_v[r, :] + md["gb"] * jnp.concatenate(acc, axis=1)).astype(BF16)
        out_copy(i).start()

    cf = c_v[...].astype(F32)
    sc = jnp.broadcast_to((cf * jax.nn.sigmoid(cf)).astype(BF16), (16, D))
    md = {}
    sch = _Sched(never)
    for i in range(0 if os.environ.get('ONLYA') else 2):
        with scope("pro_wait%d" % i):
            for c in X[i]: c.wait()
        with scope("pro_conv%d" % i):
            for fn in kv_segs(i, i): fn(None)
            for job in dft_jobs(i, i): job(sch)
            for fn in mac_segs(i, list(range(i + 1)), True, False): fn(None)
            if i == 0:
                for job in inv_jobs(): job(sch)
    with scope("pro_mod"):
        for j, n in enumerate(("sa", "ca1", "ga", "sb", "cb1")):
            wm[j].wait()
            md[n] = mod_row(j) + (1.0 if n[-1] == "1" else 0.0)
    Q[0][0].wait()
    with scope("pro_pre"):
        for fn in pre_segs(0, 0): fn(None)

    FDUR = ([320] * (2 * FC // 128) + [256] * NL) * NFC

    class Line:
        def __init__(self):
            self.items, self.marks, self.side = [], {}, []

        def mark(self, name):
            self.marks[name] = sum(1 for _, d in self.items if d)

        def wait(self, copies):
            self.items.append((lambda sch: [c.wait() for c in copies], 0))

        def jobs(self, jobs, durs=None):
            self.items += list(zip(jobs, durs or [0] * len(jobs)))

        def run(self):
            sch = _Sched(never, [d for _, d in self.items if d])
            nt = len(sch.dur)
            for segs, t0, t1, cost in self.side:
                sch.add(segs, self.marks[t0], self.marks[t1] if isinstance(t1, str) else nt - t1, cost)
            for job, _ in self.items:
                job(sch)
            assert not sch.q

    def first_two_steps():
        a0, a1 = [None] * NL, [None] * NL
        f0, f1 = ffn_jobs(0, a0), ffn_jobs(1, a1)
        ln = Line()
        c = lambda f, lo, hi: ln.jobs(f[lo:hi], FDUR[lo:hi])
        ln.jobs(inv_jobs())
        ln.wait(Q[1] + gu[0, 0]); ln.mark("a"); c(f0, 0, 4)
        ln.wait(gu[0, 1]); c(f0, 4, 8)
        ln.wait([dn[0]]); c(f0, 8, 11); ln.mark("a_"); c(f0, 11, 13)
        ln.wait(X[2]); ln.mark("b"); c(f1, 0, 13)
        ln.wait(gu[1, 0] + [dn[1]]); ln.mark("c"); ln.jobs(dft_jobs(2, 0)); c(f0, 13, 26)
        ln.wait(X[3]); ln.mark("d"); c(f1, 13, 26)
        ln.wait(gu[2, 0] + [dn[2], wm[5]] + Q[2]); ln.mark("e")
        ln.jobs([lambda sch: md.__setitem__("gb", mod_row(5))] + inv_jobs() + dft_jobs(3, 1))
        c(f0, 26, 39)
        ln.jobs([lambda sch: ffn_out(0, a0)])
        ln.wait(X[4]); ln.mark("f"); c(f1, 26, 39)
        ln.jobs([lambda sch: ffn_out(1, a1)])
        ln.side.append((pre_segs(1, 1), "a", "a_", 55))
        ln.side.append((kv_segs(2, 0), "b", "c", 150))
        ln.side.append((kv_segs(3, 1), "d", "e", 150))
        ln.side.append((kv_segs(4, 0), "f", TAIL, 150))
        ln.side.append((mac_segs(2, [0, 1, 2], True, False), "c", "e", 57))
        ln.side.append((mac_segs(3, [1, 2], False, False), "c", "e", 57))
        ln.side.append((mac_segs(3, [0, 3], True, True), "e", TAIL, 57))
        ln.side.append((pre_segs(2, 2), "e", PTAIL, 55))
        ln.run()

    def conv_step(i, carry):
        acc = [None] * NL
        ln = Line()
        ln.jobs(inv_jobs() + dft_jobs(i + 2, i % 2))
        ln.mark("a")
        ln.jobs(ffn_jobs(i, acc), FDUR)
        ln.jobs([lambda sch: ffn_out(i, acc)])
        ln.side.append((mac_segs(i + 2, list(range(NSLOT)), True, False), "a", TAIL, 57))
        ln.side.append((kv_segs(_min(i + 3, NS - 1), (i + 3) % 2), "a", TAIL, 150))
        ln.side.append((pre_segs(i + 1, i + 1), "a", PTAIL, 55))
        ln.run()
        return carry

    def ffn_step(i, carry):
        acc = [None] * NL
        ln = Line()
        ln.jobs(inv_jobs())
        ln.mark("a")
        ln.jobs(ffn_jobs(i, acc), FDUR)
        ln.jobs([lambda sch: ffn_out(i, acc)])
        ln.side.append((pre_segs(_min(i + 1, NS - 1), i + 1), "a", PTAIL, 55))
        ln.run()
        return carry

    if os.environ.get("ONLYA"):
        md["gb"] = mod_row(5)
    else:
        with scope("s01"):
            first_two_steps()
    for c in rest: c.wait()
    with scope("loopA"):
        lax.fori_loop(2, min(6, STOP), conv_step, 0)
    with scope("loopB"):
        lax.fori_loop(6, max(STOP, 6), ffn_step, 0)
    for i in range(min(STOP, NS)):
        out_copy(i).wait()


def _call(q, k, v, shk, s, dv, wg, wu, wd, c, wm):
    ff, fu, fi = (jnp.asarray(x, dtype=BF16) for x in _dft_consts())
    any_ = pl.BlockSpec(memory_space=pl.ANY)
    vm = pltpu.VMEM
    return pl.pallas_call(
        _kernel,
        in_specs=[any_] * 14 + [pl.BlockSpec(memory_space=pltpu.SMEM)],
        out_specs=any_,
        out_shape=jax.ShapeDtypeStruct((S, D), BF16),
        scratch_shapes=[
            vm((S, D), BF16), vm((HALO + S, D), BF16), vm((S, D), BF16), vm((NB, D, P), BF16),
            vm((D, FD), BF16), vm((D, FD), BF16), vm((FD, D), BF16), vm((D, 6 * D), BF16),
            vm((4, D), BF16), vm((D,), BF16), vm((1, D), BF16),
            vm((2 * P, P), BF16), vm((2 * P, P), BF16), vm((P, P), BF16),
            vm((NB + 1, 3, P, D), F32), vm((NB + 1, 3, P, D), F32), vm((2, P, D), F32), vm((2, 2 * P, D), BF16),
            vm((4, P, D), F32),
            vm((2, BM, D), BF16), vm((1, BM, D), F32),
            vm((S + BM, D), BF16), vm((S + BM, D), F32), vm((S, D), BF16),
            pltpu.SemaphoreType.DMA((72,)), pltpu.SemaphoreType.DMA((NS,)),
        ],
        compiler_params=pltpu.CompilerParams(vmem_limit_bytes=110 * 1024 * 1024),
    )(q, k, v, shk, s, dv, wg, wu, wd, c, wm, ff, fu, fi, jnp.asarray(np.zeros((1,), np.int32)))


@jax.jit
def pallas_adaLN_cond__ssm_conv_h3__glu_gated_bilinear__prompt_kernel(
        A_q, A_k, A_v, A_shift_k, A_ssm_k, A_ssm_D, B_x, B_w_gate, B_w_up, B_w_down, c, w_mod):
    out = _call(A_q.reshape(S, D), A_k.reshape(S, D), A_v.reshape(S, D), A_shift_k.T, A_ssm_k,
                A_ssm_D, B_w_gate, B_w_up, B_w_down, c, w_mod)
    return out.reshape(1, S, D)
```

```python
import numpy as np
import jax
import jax.numpy as jnp
from jax import lax
import jax.experimental.pallas as pl
import jax.experimental.pallas.tpu as pltpu

S, D, FD = 2048, 640, 1536
P = 128
NB = S // P
BM = 256
NS = S // BM
NL = D // 128
HALO = 16
EPS = 1e-5
F32, BF16 = jnp.float32, jnp.bfloat16
FC = 512
NFC = FD // FC
TAIL, PTAIL = 1, 4
PRE_LAG = 4
KVR = 64


def _dft_consts():
    f = np.concatenate([np.arange(0, P, 2), np.arange(1, P, 2)]).astype(np.float64)
    w = np.pi * (2 * f[:, None] + 1) / (2 * P)
    n = np.arange(P, dtype=np.float64)[None, :]
    mid = (P - 1) / 2
    fk = np.concatenate([np.cos(w * n), -np.sin(w * n)], axis=0)
    fu = np.concatenate([np.cos(w * (n - mid)), -np.sin(w * (n - mid))], axis=0)
    tau = n[:, P // 2:] - mid
    fi = np.concatenate([np.cos(w * tau).T, np.sin(w * tau).T], axis=0) / P
    return fk.astype(np.float32), fu.astype(np.float32), fi.astype(np.float32)


def _al(x, m):
    return x if isinstance(x, int) else pl.multiple_of(x, m)


def _rows(start, n, m=16):
    return pl.ds(_al(start, m), n)


def _min(a, b):
    return min(a, b) if isinstance(a, int) else jnp.minimum(a, b)


class _Sched:
    def __init__(self, mask, dur=()):
        self.mask = mask
        self.dur = list(dur)
        self.load = [0.0] * len(self.dur)
        self.q = {}
        self.t = 0

    def add(self, segs, t0, t1, cost):
        total = cost * len(segs)
        lo, hi = 0.0, 1e3
        for _ in range(50):
            mid = (lo + hi) / 2
            room = sum(max(0.0, mid * self.dur[t] - self.load[t]) for t in range(t0, t1))
            lo, hi = (lo, mid) if room >= total else (mid, hi)
        t, left = t0, max(0.0, hi * self.dur[t0] - self.load[t0])
        for fn in segs:
            while left < cost / 2 and t + 1 < t1:
                t += 1
                left += max(0.0, hi * self.dur[t] - self.load[t])
            self.q.setdefault(t, []).append(fn)
            self.load[t] += cost
            left -= cost

    def fire(self, p):
        segs = self.q.pop(self.t, [])
        self.t += 1
        nrg, nlt = p.shape[0] // 8, p.shape[1] // 128
        for j, fn in enumerate(segs):
            rg = (j * nrg) // len(segs)
            lt = j % min(nlt, 4)
            fn(jnp.where(self.mask, p[rg * 8:rg * 8 + 8, lt * 128:(lt + 1) * 128], 0.0))


def _kernel(q_h, k_h, v_h, shk_h, s_h, dv_h, wg_h, wu_h, wd_h, c_h, wm_h, ff_h, fu_h, fi_h, z_s, o_h,
            q_v, k_v, v_v, s_v, wg_v, wu_v, wd_v, wm_v, shk_v, dv_v, c_v, ff_v, fu_v, fi_v,
            K_s, W_s, Zl_s, Z_s, Zp_s, kv_s, y_s, hb_v, x1_v, o_v, sems, osem, tsem):
    nsem = [0]

    def mk(src, dst):
        c = pltpu.make_async_copy(src, dst, sems.at[nsem[0]])
        nsem[0] += 1
        return c

    def qq(i):
        r = pl.ds(i * BM, BM)
        return [mk(q_h.at[r], q_v.at[r])]

    def skv(i):
        r = pl.ds(i * BM, BM)
        return ([mk(s_h.at[:, pl.ds((2 * i + b) * P, P)], s_v.at[2 * i + b]) for b in range(2)]
                + [mk(k_h.at[r], k_v.at[pl.ds(HALO + i * BM, BM)]), mk(v_h.at[r], v_v.at[r])])

    def out_copy(i):
        r = _rows(i * BM, BM)
        return pltpu.make_async_copy(o_v.at[r], o_h.at[r], osem.at[i])

    def out_tile(i, n):
        r, cs = _rows(i * BM, BM), pl.ds(n * 128, 128)
        return pltpu.make_async_copy(o_v.at[r, cs], o_h.at[r, cs], tsem.at[i - 6, n])

    small = [mk(shk_h, shk_v), mk(dv_h, dv_v), mk(c_h, c_v), mk(ff_h, ff_v), mk(fu_h, fu_v), mk(fi_h, fi_v)]
    Q = [qq(i) for i in range(NS)]
    X = [skv(i) for i in range(NS)]
    wm = [mk(wm_h.at[:, pl.ds(j * D, D)], wm_v.at[:, pl.ds(j * D, D)]) for j in range(6)]
    gu = {}
    for j in range(NFC):
        for h in range(2 if j == 0 else 1):
            cs = pl.ds(j * FC + h * FC // 2, FC // 2 if j == 0 else FC)
            gu[j, h] = [mk(wg_h.at[:, cs], wg_v.at[:, cs]), mk(wu_h.at[:, cs], wu_v.at[:, cs])]
    dn = [mk(wd_h.at[pl.ds(j * FC, FC)], wd_v.at[pl.ds(j * FC, FC)]) for j in range(NFC)]

    order = (small + X[0] + X[1] + wm[:5] + Q[0] + Q[1] + gu[0, 0] + gu[0, 1] + [dn[0]] + X[2] + gu[1, 0] + [dn[1]]
             + X[3] + gu[2, 0] + [dn[2], wm[5]] + Q[2] + X[4] + Q[3])
    for i in range(4, NS):
        order += Q[i] + (X[i + 1] if i + 1 < NS else [])
    for c in order:
        c.start()
    rest = [c for i in range(3, NS) for c in Q[i]] + [c for i in range(5, NS) for c in X[i]]

    k_v[0:HALO, :] = jnp.zeros((HALO, D), BF16)
    z0 = z_s[0]
    K_s[NB + z0] = jnp.zeros((2, P, D), F32)
    W_s[NB + z0] = jnp.zeros((3, P, D), F32)

    for c in small: c.wait()
    ff, fu = ff_v[...], fu_v[...]
    fic, fis = fi_v[0:P // 2, :], fi_v[P // 2:, :]
    never = ff_v[0:8, :].astype(F32) > 2.0
    rev8 = 7 - lax.broadcasted_iota(jnp.int32, (8, 128), 0)
    taps = shk_v[...].astype(F32)
    dvec = dv_v[...].astype(F32).reshape(1, D)

    def kv_segs(i, slot):
        segs = []
        R = KVR
        for l in range(NL):
            ls = slice(l * 128, (l + 1) * 128)
            for r in range(0, BM, R):
                def seg(trig, ls=ls, r=r):
                    kk = k_v[_rows(i * BM + r + HALO - 8, 8 + R, 8), ls].astype(F32)
                    acc = kk[8:, :] * taps[0:1, ls]
                    if trig is not None:
                        acc = acc + jnp.concatenate([trig] * (R // 8), axis=0)
                    for j in range(1, 4):
                        acc = acc + pltpu.roll(kk, j, axis=0)[8:, :] * taps[j:j + 1, ls]
                    kv_s[slot, r:r + R, ls] = (acc * v_v[_rows(i * BM + r, R), ls].astype(F32)).astype(BF16)
                segs.append(seg)
        return segs

    def mac_segs(j, ts, final, resume):
        segs = []
        static = isinstance(j, int)

        def kidx(t, e):
            return 2 * t + e if static or t <= 4 else jnp.where(t <= j, 2 * t + e, NB)

        def widx(t, d):
            a = 2 * (j - t) + d
            if static:
                return a if a >= 0 else None
            return a if (t <= 4 and d >= 0) or t < 4 else jnp.where(a >= 0, a, NB)
        kix = {(t, e): kidx(t, e) for t in ts for e in range(2)}
        wix = {(t, d): widx(t, d) for t in ts for d in (-1, 0, 1)}
        for l in range(NL):
            ls = slice(l * 128, (l + 1) * 128)
            for r2 in range(P // 16):
                sts = [dict(), dict()]
                for gi, t in enumerate(ts):
                    def seg(trig, ls=ls, r2=r2, t=t, sts=sts, last=gi == len(ts) - 1):
                        outv = [[], []]
                        for h in range(2):
                            rows = slice((2 * r2 + h) * 8, (2 * r2 + h) * 8 + 8)
                            acc = sts[h]
                            ww = {d: [W_s[wix[t, d], x, rows, ls] for x in range(3)]
                                  for d in (-1, 0, 1) if wix[t, d] is not None}
                            for e in range(2):
                                ka, kb = [K_s[kix[t, e], x, rows, ls] for x in range(2)]
                                if trig is not None:
                                    ka = ka + trig
                                kk = [ka + kb, ka, kb]
                                for b in range(2):
                                    if b - e in ww:
                                        pr = [kk[x] * ww[b - e][x] for x in range(3)]
                                        acc[b] = pr if b not in acc else [acc[b][x] + pr[x] for x in range(3)]
                            if not last:
                                continue
                            z = []
                            for b in range(2):
                                re, im = acc[b][0] - acc[b][2], acc[b][0] + acc[b][1]
                                if resume:
                                    re = re + Zp_s[2 * b + z0, rows, ls]
                                    im = im + Zp_s[2 * b + 1 + z0, rows, ls]
                                z.append((re, im))
                            if final:
                                def shifted(cur, prev):
                                    if (2 * r2 + h) * 8 < P // 2:
                                        return cur[0] - prev[1], cur[1] + prev[0]
                                    return cur[0] + prev[1], cur[1] - prev[0]
                                z1 = shifted(z[1], z[0])
                                if static and j == 0:
                                    z0v = z[0]
                                else:
                                    z0v = shifted(z[0], (Zl_s[z0, rows, ls], Zl_s[1 + z0, rows, ls]))
                                Zl_s[z0, rows, ls] = z[1][0]
                                Zl_s[1 + z0, rows, ls] = z[1][1]
                                z = [z0v, z1]
                            for b in range(2):
                                outv[b].append(z[b])
                        if last:
                            rows = slice(r2 * 16, r2 * 16 + 16)
                            for b in range(2):
                                for x in range(2):
                                    val = jnp.concatenate([outv[b][0][x], outv[b][1][x]], axis=0)
                                    if final:
                                        Z_s[b + z0, x * P + r2 * 16:x * P + r2 * 16 + 16, ls] = val.astype(BF16)
                                    else:
                                        Zp_s[2 * b + x + z0, rows, ls] = val
                    segs.append(seg)
        return segs

    def tie(x, trig):
        if trig is None:
            return x
        t = jnp.concatenate([trig] * (x.shape[0] // 8), axis=0)
        return jnp.concatenate([x[:, :128] + t, x[:, 128:]], axis=1)

    def pre_segs(i, dst):
        R = 16
        chains = []
        for r in range(0, BM, R):
            st = {}

            def a(trig, r=r, st=st):
                st["x"] = tie(q_v[_rows(i * BM + r, R), :].astype(F32), trig)
                st["m"] = jnp.mean(st["x"], axis=-1, keepdims=True)

            def b(trig, st=st):
                st["xc"] = tie(st["x"], trig) - st["m"]
                st["v"] = jnp.mean(st["xc"] * st["xc"], axis=-1, keepdims=True)

            def c(trig, r=r, st=st):
                h = tie(st["xc"], trig) * lax.rsqrt(st["v"] + EPS) * md["ca1"] + md["sa"]
                st["x1"] = st["x"] + md["ga"] * (h * y_s[z0, r:r + R, :])
                x1_v[_rows(dst * BM + r, R), :] = st["x1"]
                st["m1"] = jnp.mean(st["x1"], axis=-1, keepdims=True)

            def d(trig, st=st):
                st["xc1"] = tie(st["x1"], trig) - st["m1"]
                st["v1"] = jnp.mean(st["xc1"] * st["xc1"], axis=-1, keepdims=True)

            def e(trig, r=r, st=st):
                hb = tie(st["xc1"], trig) * lax.rsqrt(st["v1"] + EPS) * md["cb1"] + md["sb"]
                hb_v[_rows(dst * BM + r, R), :] = hb.astype(BF16)
            chains.append([a, b, c, d, e])
        order = sorted((g + PRE_LAG * s, -s, g) for g in range(len(chains)) for s in range(5))
        return [chains[g][-ns] for _, ns, g in order]

    def dft_jobs(i, slot):
        def kjob(sch, b):
            a = 2 * i + b
            Kf = lax.dot_general(ff, s_v[a], (((1,), (1,)), ((), ())), preferred_element_type=F32)
            kr, ki = Kf[0:P], Kf[P:]
            if isinstance(a, int) and a == 0:
                kr = kr + dvec
            K_s[a + z0, 0] = kr
            K_s[a + z0, 1] = ki

        def ujob(sch, b):
            a = 2 * i + b
            U = jnp.dot(fu, kv_s[slot, b * P:(b + 1) * P, :], preferred_element_type=F32)
            wr, wi = U[0:P], U[P:]
            W_s[a + z0, 0] = wr
            W_s[a + z0, 1] = wi - wr
            W_s[a + z0, 2] = wr + wi
        return [lambda sch, b=b, f=f: f(sch, b) for f in (kjob, ujob) for b in range(2)]

    def inv_jobs():
        def job(sch, b):
            ye = jnp.dot(fic, Z_s[b + z0, 0:P, :], preferred_element_type=F32)
            yo = jnp.dot(fis, Z_s[b + z0, P:2 * P, :], preferred_element_type=F32)
            y_s[z0, b * P + P // 2:(b + 1) * P, :] = ye - yo
            lo = ye + yo
            for g in range(P // 16):
                src = slice((P // 16 - 1 - g) * 8, (P // 16 - g) * 8)
                y_s[z0, b * P + g * 8:b * P + g * 8 + 8, :] = jnp.concatenate(
                    [jnp.take_along_axis(lo[src, l * 128:(l + 1) * 128], rev8, axis=0) for l in range(NL)], axis=1)
        return [lambda sch, b=b: job(sch, b) for b in range(2)]

    def mod_row(j):
        r = jnp.dot(sc, wm_v[:, j * D:(j + 1) * D], preferred_element_type=F32)
        return r[0:1, :]

    def ffn_jobs(i, acc):
        st = {}
        jobs = []
        for j in range(NFC):
            for n in range(FC // 128):
                cs = slice(j * FC + n * 128, j * FC + (n + 1) * 128)

                def gate(sch, j=j, n=n, cs=cs):
                    if n == 0:
                        st["hh"] = []
                        if j == 0:
                            st["hb"] = hb_v[_rows(i * BM, BM), :]
                    st["g"] = jnp.dot(st["hb"], wg_v[:, cs], preferred_element_type=F32)
                    sch.fire(st["g"])

                def up(sch, cs=cs):
                    u = jnp.dot(st["hb"], wu_v[:, cs], preferred_element_type=F32)
                    sch.fire(u)
                    st["hh"].append(st["g"] * u)
                jobs += [gate, up]
            for n in range(NL):
                def down(sch, j=j, n=n):
                    if n == 0:
                        st["h"] = jnp.concatenate(st["hh"], axis=1).astype(BF16)
                    t = jnp.dot(st["h"], wd_v[j * FC:(j + 1) * FC, n * 128:(n + 1) * 128], preferred_element_type=F32)
                    sch.fire(t)
                    acc[n] = t if acc[n] is None else acc[n] + t
                jobs.append(down)
        return jobs

    def ffn_out(i, acc):
        r = _rows(i * BM, BM)
        o_v[r, :] = (x1_v[r, :] + md["gb"] * jnp.concatenate(acc, axis=1)).astype(BF16)
        out_copy(i).start()

    cf = c_v[...].astype(F32)
    sc = jnp.broadcast_to((cf * jax.nn.sigmoid(cf)).astype(BF16), (16, D))
    md = {}
    sch = _Sched(never)
    for i in range(2):
        for c in X[i]: c.wait()
        for fn in kv_segs(i, i): fn(None)
        for job in dft_jobs(i, i): job(sch)
        for fn in mac_segs(i, list(range(i + 1)), True, False): fn(None)
        if i == 0:
            for job in inv_jobs(): job(sch)
    for j, n in enumerate(("sa", "ca1", "ga", "sb", "cb1")):
        wm[j].wait()
        md[n] = mod_row(j) + (1.0 if n[-1] == "1" else 0.0)
    Q[0][0].wait()
    for fn in pre_segs(0, 0): fn(None)

    FDUR = ([320] * (2 * FC // 128) + [256] * NL) * NFC

    class Line:
        def __init__(self):
            self.items, self.marks, self.side = [], {}, []

        def mark(self, name):
            self.marks[name] = sum(1 for _, d in self.items if d)

        def wait(self, copies):
            self.items.append((lambda sch: [c.wait() for c in copies], 0))

        def jobs(self, jobs, durs=None):
            self.items += list(zip(jobs, durs or [0] * len(jobs)))

        def run(self):
            sch = _Sched(never, [d for _, d in self.items if d])
            nt = len(sch.dur)
            for segs, t0, t1, cost in self.side:
                sch.add(segs, self.marks[t0], self.marks[t1] if isinstance(t1, str) else nt - t1, cost)
            for job, _ in self.items:
                job(sch)
            assert not sch.q

    def first_two_steps():
        a0, a1 = [None] * NL, [None] * NL
        f0, f1 = ffn_jobs(0, a0), ffn_jobs(1, a1)
        ln = Line()
        c = lambda f, lo, hi: ln.jobs(f[lo:hi], FDUR[lo:hi])
        ln.jobs(inv_jobs())
        ln.wait(Q[1] + gu[0, 0]); ln.mark("a"); c(f0, 0, 4)
        ln.wait(gu[0, 1]); c(f0, 4, 8)
        ln.wait([dn[0]]); c(f0, 8, 11); ln.mark("a_"); c(f0, 11, 13)
        ln.wait(X[2]); ln.mark("b"); c(f1, 0, 13)
        ln.wait(gu[1, 0] + [dn[1]]); ln.mark("c"); ln.jobs(dft_jobs(2, 0)); c(f0, 13, 26)
        ln.wait(X[3]); ln.mark("d"); c(f1, 13, 26)
        ln.wait(gu[2, 0] + [dn[2], wm[5]] + Q[2]); ln.mark("e")
        ln.jobs([lambda sch: md.__setitem__("gb", mod_row(5))] + inv_jobs() + dft_jobs(3, 1))
        c(f0, 26, 39)
        ln.jobs([lambda sch: ffn_out(0, a0)])
        ln.wait(X[4]); ln.mark("f"); c(f1, 26, 39)
        ln.jobs([lambda sch: ffn_out(1, a1)])
        ln.side.append((pre_segs(1, 1), "a", "a_", 55))
        ln.side.append((kv_segs(2, 0), "b", "c", 150))
        ln.side.append((kv_segs(3, 1), "d", "e", 150))
        ln.side.append((kv_segs(4, 0), "f", TAIL, 150))
        ln.side.append((mac_segs(2, [0, 1, 2], True, False), "c", "e", 57))
        ln.side.append((mac_segs(3, [1, 2], False, False), "c", "e", 57))
        ln.side.append((mac_segs(3, [0, 3], True, True), "e", TAIL, 57))
        ln.side.append((pre_segs(2, 2), "e", PTAIL, 55))
        ln.run()

    def conv_step(i, carry):
        acc = [None] * NL
        ln = Line()
        ln.jobs(inv_jobs() + dft_jobs(i + 2, i % 2))
        ln.mark("a")
        ln.jobs(ffn_jobs(i, acc), FDUR)
        ln.jobs([lambda sch: ffn_out(i, acc)])
        ln.side.append((mac_segs(i + 2, list(range(NS)), True, False), "a", TAIL, 57))
        ln.side.append((kv_segs(_min(i + 3, NS - 1), (i + 3) % 2), "a", TAIL, 150))
        ln.side.append((pre_segs(i + 1, i + 1), "a", PTAIL, 55))
        ln.run()
        return carry

    def ffn_step(i, carry):
        acc = [None] * NL
        ln = Line()
        ln.jobs(inv_jobs())
        ln.mark("a")
        jobs = ffn_jobs(i, acc)
        for t, job in enumerate(jobs):
            ln.jobs([job], [FDUR[t]])
            n = t - (len(jobs) - NL)
            if n >= 0:
                def out(sch, n=n):
                    r, cs = _rows(i * BM, BM), pl.ds(n * 128, 128)
                    o_v[r, cs] = (x1_v[r, cs] + md["gb"][:, n * 128:(n + 1) * 128] * acc[n]).astype(BF16)
                    out_tile(i, n).start()
                ln.jobs([out])
        ln.side.append((pre_segs(_min(i + 1, NS - 1), i + 1), "a", PTAIL, 55))
        ln.run()
        return carry

    first_two_steps()
    for c in rest: c.wait()
    lax.fori_loop(2, 6, conv_step, 0)
    lax.fori_loop(6, NS, ffn_step, 0)
    for i in range(6):
        out_copy(i).wait()
    for i in range(6, NS):
        for n in range(NL):
            out_tile(i, n).wait()


def _call(q, k, v, shk, s, dv, wg, wu, wd, c, wm):
    ff, fu, fi = (jnp.asarray(x, dtype=BF16) for x in _dft_consts())
    any_ = pl.BlockSpec(memory_space=pl.ANY)
    vm = pltpu.VMEM
    return pl.pallas_call(
        _kernel,
        in_specs=[any_] * 14 + [pl.BlockSpec(memory_space=pltpu.SMEM)],
        out_specs=any_,
        out_shape=jax.ShapeDtypeStruct((S, D), BF16),
        scratch_shapes=[
            vm((S, D), BF16), vm((HALO + S, D), BF16), vm((S, D), BF16), vm((NB, D, P), BF16),
            vm((D, FD), BF16), vm((D, FD), BF16), vm((FD, D), BF16), vm((D, 6 * D), BF16),
            vm((4, D), BF16), vm((D,), BF16), vm((1, D), BF16),
            vm((2 * P, P), BF16), vm((2 * P, P), BF16), vm((P, P), BF16),
            vm((NB + 1, 2, P, D), F32), vm((NB + 1, 3, P, D), F32), vm((2, P, D), F32), vm((2, 2 * P, D), BF16),
            vm((4, P, D), F32),
            vm((2, BM, D), BF16), vm((1, BM, D), F32),
            vm((S + BM, D), BF16), vm((S + BM, D), F32), vm((S, D), BF16),
            pltpu.SemaphoreType.DMA((72,)), pltpu.SemaphoreType.DMA((NS,)), pltpu.SemaphoreType.DMA((2, NL)),
        ],
        compiler_params=pltpu.CompilerParams(vmem_limit_bytes=110 * 1024 * 1024),
    )(q, k, v, shk, s, dv, wg, wu, wd, c, wm, ff, fu, fi, jnp.asarray(np.zeros((1,), np.int32)))


@jax.jit
def pallas_adaLN_cond__ssm_conv_h3__glu_gated_bilinear__prompt_kernel(
        A_q, A_k, A_v, A_shift_k, A_ssm_k, A_ssm_D, B_x, B_w_gate, B_w_up, B_w_down, c, w_mod):
    out = _call(A_q.reshape(S, D), A_k.reshape(S, D), A_v.reshape(S, D), A_shift_k.T, A_ssm_k,
                A_ssm_D, B_w_gate, B_w_up, B_w_down, c, w_mod)
    return out.reshape(1, S, D)
```
